```python
import os as _os
_os.environ.setdefault("JAX_PLATFORMS", "cpu")
import jax
import jax.numpy as jnp

def _softmax(x, axis=-1):
    return jax.nn.softmax(x, axis=axis)
def _gelu(x):
    return jax.nn.gelu(x, approximate=True)
def _silu(x):
    return jax.nn.silu(x)
def _sigmoid(x):
    return jax.nn.sigmoid(x)
def _layernorm(x, axis=-1, eps=1e-5):
    m = jnp.mean(x, axis=axis, keepdims=True)
    v = jnp.var(x, axis=axis, keepdims=True)
    return (x - m) / jnp.sqrt(v + eps)
def _scatter_add(tgt, idx, src, axis=0):
    return tgt.at[idx].add(src)
def _segment_sum(src, seg, n):
    return jax.ops.segment_sum(src, seg, n)
class _Rng:
    def __init__(self, key):
        self._k = key
    def _next(self):
        self._k, sub = jax.random.split(self._k)
        return sub
    def normal(self, shape):
        return jax.random.normal(self._next(), shape, dtype=jnp.bfloat16)
    def randint(self, lo, hi, shape):
        return jax.random.randint(self._next(), shape, lo, hi, dtype=jnp.int32)
    def uniform(self, shape, lo=0.0, hi=1.0):
        return jax.random.uniform(self._next(), shape, jnp.bfloat16, lo, hi)
    def permutation(self, n):
        return jax.random.permutation(self._next(), n)


kernel_name = 'standalone__sliding_block_cached__sampling'

def setup_inputs():
    _rng = _Rng(jax.random.key(int.from_bytes(__import__("os").urandom(4), "little")))
    _w = (lambda a: (lambda t: t.astype(jnp.bfloat16) if jnp.issubdtype(t.dtype, jnp.floating) else t)(jnp.asarray(a)))
    B, Sq, D = 8, 16, 576
    Hq, Hkv, Sk, Dh = 32, 16, 8192, 128
    assert Hq % Hkv == 0, (Hq, Hkv)
    return {
        "x": _w((lambda *s: _rng.normal(s) * 0.8)(B, Sq, D)),
        "k_cache": _w((lambda *s: _rng.normal(s) * 0.8)(B, Hkv, Sk, Dh)),
        "v_cache": _w((lambda *s: _rng.normal(s) * 0.05)(B, Hkv, Sk, Dh)),
        "wq": _w((lambda *s: _rng.normal(s) * 0.8)(D, Hq * Dh) * (D ** -0.5)),
        "wo": _w((lambda *s: _rng.normal(s) * 0.05)(Hq * Dh, D) * ((Hq * Dh) ** -0.5)),
    }

def reference(x, k_cache, v_cache, wq, wo):
    B, Sq, D = x.shape
    Hq, Dh = 32, 128
    Hkv, Sk = k_cache.shape[1], k_cache.shape[2]
    W = min(4096, max(256, Sk // 4))
    rep = Hq // Hkv
    q = (lambda x, *d: x.transpose(*d))((x @ wq).reshape(B, Sq, Hq, Dh), 0, 2, 1, 3)
    k = jnp.repeat(k_cache[:, :, Sk - W:, :], rep, axis=1)
    v = jnp.repeat(v_cache[:, :, Sk - W:, :], rep, axis=1)
    scores = jnp.einsum("bhqd,bhkd->bhqk", q, k) * (Dh ** -0.5)
    p = _softmax(scores, axis=-1)
    o = jnp.einsum("bhqk,bhkd->bhqd", p, v)
    return (lambda x, *d: x.transpose(*d))(o, 0, 2, 1, 3).reshape(B, Sq, Hq * Dh) @ wo
```

```python
import math

import jax
import jax.numpy as jnp
from jax import lax
import jax.experimental.pallas as pl
import jax.experimental.pallas.tpu as pltpu

_HQ, _DH = 32, 128
_NT = (((1,), (1,)), ((), ()))

_ROWS = 128
_DMA_ELEMS = _ROWS * _DH
_NW = 4
_NSLOT = 16
_LOOKAHEAD = 3


@jax.jit
def pallas_standalone__sliding_block_cached__sampling_kernel(
    x: jax.Array,
    k_cache: jax.Array,
    v_cache: jax.Array,
    wq: jax.Array,
    wo: jax.Array,
):
    B, SQ, D = x.shape
    _, HKV, SK, _ = k_cache.shape
    W = min(4096, max(256, SK // 4))
    REP = _HQ // HKV
    M = B * SQ
    E = _HQ * _DH
    NP = B * HKV
    NC = W // _ROWS
    NB = pl.cdiv(D, 128)
    DP = NB * 128
    EDGE = D - (NB - 1) * 128
    exp_scale = (_DH ** -0.5) * math.log2(math.e)

    pieces = [((NB - 1) * 128, EDGE, 0, E), (0, 128, 0, E)]
    for n in range(1, NB - 2):
        pieces += [(n * 128, 128, c, E // 2) for c in range(0, E, E // 2)]
    pieces += [((NB - 2) * 128, 128, c, E // 4) for c in range(0, E, E // 4)]

    def kernel(x_hbm, k_hbm, v_hbm, wq_hbm, wot_hbm, o_hbm,
               x_v, wq_v, wo_v, kv_v, q_v, a_v, o_v, sem_in, sem_wo, sem_kv, sem_o):

        def kv_chunk(p, c):
            slot = lax.rem(p, _NSLOT)
            r = pl.multiple_of(c * _ROWS, _ROWS)
            for t, src in enumerate((k_hbm, v_hbm)):
                pltpu.make_async_copy(src.at[p, pl.ds(SK - W + r, _ROWS), :],
                                      kv_v.at[slot, t, pl.ds(r, _ROWS), :],
                                      sem_kv.at[slot]).start(priority=t)

        def kv_issue(s):
            part = lax.rem(s + _NW, _NW)

            @pl.loop(0, NC // (2 * _NW))
            def _(e):
                for j in range(_NW):
                    p = s + lax.rem(j - s + _NW * NP, _NW)

                    @pl.when((p >= 0) & (p < NP))
                    def _():
                        for c0 in range(2):
                            kv_chunk(p, c0 + 2 * part + 2 * _NW * e)

        def weight_copies(src, dst, r0, rows, c0, cols, sem):
            nc = min(cols, E // 2)
            nr = _DMA_ELEMS // nc
            return [(src.at[pl.ds(r, nr), pl.ds(c, nc)], dst.at[pl.ds(r, nr), pl.ds(c, nc)], sem)
                    for r in range(r0, r0 + rows, nr) for c in range(c0, c0 + cols, nc)]

        def start_all(copies):
            for i, c in enumerate(copies):
                pltpu.make_async_copy(*c).start(priority=i % 2)

        x_copy = pltpu.make_async_copy(x_hbm, x_v, sem_in.at[0])
        x_copy.start()
        wq_copies = weight_copies(wq_hbm, wq_v, 0, D, 0, E, sem_in.at[1])
        order = [u * 16 + c0 + 2 * q + 8 * e for q in range(4) for e in range(2) for j in range(4)
                 for c0 in range(2) for u in (j, j + 4)]
        start_all([wq_copies[i] for i in order] + wq_copies[len(order):])

        if DP > D:
            wo_v[D:DP, :] = jnp.zeros((DP - D, E), wo_v.dtype)

        @pl.loop(1 - _NW, _LOOKAHEAD)
        def _(s):
            kv_issue(s)

        x_copy.wait()
        pltpu.make_async_copy(wq_v, wq_v, sem_in.at[1]).wait()

        def q_projection(g):
            col = pl.multiple_of(g * (REP * _DH), REP * _DH)
            q = jnp.dot(x_v[...], wq_v[:, pl.ds(col, REP * _DH)], preferred_element_type=jnp.float32)
            q = q.astype(q_v.dtype)
            for r in range(REP):
                for b in range(B):
                    q_v[b, g, r * SQ:(r + 1) * SQ, :] = q[b * SQ:(b + 1) * SQ, r * _DH:(r + 1) * _DH]

        def attend(slot, b, g):
            s = lax.dot_general(q_v[b, g], kv_v[slot, 0], _NT, preferred_element_type=jnp.float32)
            m = jnp.max(s, axis=-1, keepdims=True)
            p = jnp.exp2((s - m) * exp_scale)
            l = jnp.sum(p, axis=-1, keepdims=True)
            o = jnp.dot(p.astype(kv_v.dtype), kv_v[slot, 1], preferred_element_type=jnp.float32)
            o = (o / l).astype(a_v.dtype)
            row = pl.multiple_of(b * SQ, SQ)
            for r in range(REP):
                a_v[g * REP + r, pl.ds(row, SQ), :] = o[r * SQ:(r + 1) * SQ, :]

        wo_copies, wo_end = [], []
        for u, piece in enumerate(pieces):
            wo_copies += weight_copies(wot_hbm, wo_v, *piece, sem_wo.at[u])
            wo_end.append(len(wo_copies))
        wo_sched = (16, 32, 32)
        first_tail = NP - _NW + 1

        @pl.loop(0, NP)
        def _(i):
            s = i + _LOOKAHEAD

            @pl.loop(s, jnp.where(s < first_tail, s + 1, jnp.where(s == first_tail, NP, s)))
            def _(ss):
                kv_issue(ss)

            @pl.when(i < HKV)
            def _():
                q_projection(i)

            slot = lax.rem(i, _NSLOT)
            pltpu.make_async_copy(kv_v.at[slot], kv_v.at[slot], sem_kv.at[slot]).wait()
            done = 0
            for t, n in enumerate(wo_sched):
                @pl.when(i == NP - len(wo_sched) + t)
                def _():
                    start_all(wo_copies[done:done + n])
                done += n
            attend(slot, lax.div(i, HKV), lax.rem(i, HKV))

        issued = sum(wo_sched)
        acc = None
        for u, (r0, rows, c0, cols) in enumerate(pieces):
            upto = min(len(wo_copies), wo_end[u] + 64)
            if upto > issued:
                start_all(wo_copies[issued:upto])
                issued = upto
            blk = wo_v.at[pl.ds(r0, rows), pl.ds(c0, cols)]
            pltpu.make_async_copy(blk, blk, sem_wo.at[u]).wait()
            for h in range(c0 // _DH, (c0 + cols) // _DH):
                t = lax.dot_general(a_v[h], wo_v[r0:r0 + rows, h * _DH:(h + 1) * _DH], _NT,
                                    preferred_element_type=jnp.float32)
                acc = t if acc is None else acc + t
            if c0 + cols == E:
                o_v[:, r0:r0 + rows] = acc.astype(o_v.dtype)
                acc = None
                pltpu.make_async_copy(o_v.at[:, pl.ds(r0, rows)], o_hbm.at[:, pl.ds(r0, rows)], sem_o).start()

        pltpu.make_async_copy(o_v, o_hbm, sem_o).wait()

    hbm = pl.BlockSpec(memory_space=pltpu.HBM)
    out = pl.pallas_call(
        kernel,
        out_shape=jax.ShapeDtypeStruct((M, D), x.dtype),
        in_specs=[hbm] * 5,
        out_specs=hbm,
        scratch_shapes=[
            pltpu.VMEM((M, D), x.dtype),
            pltpu.VMEM((D, E), wq.dtype),
            pltpu.VMEM((DP, E), wo.dtype),
            pltpu.VMEM((_NSLOT, 2, W, _DH), k_cache.dtype),
            pltpu.VMEM((B, HKV, REP * SQ, _DH), k_cache.dtype),
            pltpu.VMEM((_HQ, M, _DH), wo.dtype),
            pltpu.VMEM((M, D), x.dtype),
            pltpu.SemaphoreType.DMA((2,)),
            pltpu.SemaphoreType.DMA((len(pieces),)),
            pltpu.SemaphoreType.DMA((_NSLOT,)),
            pltpu.SemaphoreType.DMA(()),
        ],
        compiler_params=pltpu.CompilerParams(
            vmem_limit_bytes=100 * 1024 * 1024,
            disable_bounds_checks=True,
            disable_semaphore_checks=True,
        ),
        name="sliding_block_cached_sampling",
    )(x.reshape(M, D), k_cache.reshape(NP, SK, _DH), v_cache.reshape(NP, SK, _DH), wq, wo.T)
    return out.reshape(B, SQ, D)
```

```python
import math

import jax
import jax.numpy as jnp
from jax import lax
import jax.experimental.pallas as pl
import jax.experimental.pallas.tpu as pltpu

_HQ, _DH = 32, 128
_NT = (((1,), (1,)), ((), ()))

_ROWS = 128
_WIDTH = 4
_WINDOW_ORDER = (0, 2, 1, 3)
_V_LEAD = 3
_LOOKAHEAD = 2
_SLOTS = 16
_QUEUE1_LAG = 30


@jax.jit
def pallas_standalone__sliding_block_cached__sampling_kernel(
    x: jax.Array,
    k_cache: jax.Array,
    v_cache: jax.Array,
    wq: jax.Array,
    wo: jax.Array,
):
    B, SQ, D = x.shape
    _, HKV, SK, _ = k_cache.shape
    W = min(4096, max(256, SK // 4))
    REP = _HQ // HKV
    M = B * SQ
    E = _HQ * _DH
    PAIRS = B * HKV
    CHUNKS = W // _ROWS
    assert W % (2 * _WIDTH * _ROWS) == 0 and D == 576 and PAIRS >= _SLOTS
    assert _SLOTS > _LOOKAHEAD + _V_LEAD + _WIDTH
    exp2_scale = (_DH ** -0.5) * math.log2(math.e)

    wo_pieces = [
        (row, rows, E * a // 4, E * (b - a) // 4)
        for row, rows, cuts in ((512, 64, (0, 4)), (0, 128, (0, 4)), (128, 128, (0, 2, 4)),
                                (256, 128, (0, 2, 4)), (384, 128, (0, 2, 3, 4)))
        for a, b in zip(cuts, cuts[1:])
    ]

    def kernel(x_hbm, k_hbm, v_hbm, wq_hbm, wot_hbm, out_hbm,
               x_ref, wq_ref, wot_ref, kv_ref, q_ref, att_ref, out_ref, x_sem, sems, out_sems):
        WQ_SEM, WO_SEM = _SLOTS, _SLOTS + 1

        def kv_copy(which, pair, chunk, zero=0):
            static = isinstance(pair, int)
            slot = pair % _SLOTS if static else lax.rem(pair, _SLOTS)
            row = chunk * _ROWS if static else pl.multiple_of(chunk * _ROWS, _ROWS)
            return pltpu.make_async_copy(
                (k_hbm, v_hbm)[which].at[pair, pl.ds(SK - W + row, _ROWS), :],
                kv_ref.at[slot, which, pl.ds(row, _ROWS), :],
                sems.at[slot + zero])

        def weight_copy(src, dst, row, rows, col, cols, sem, zero=0):
            block = (pl.ds(row, rows), pl.ds(col, cols))
            return pltpu.make_async_copy(src.at[block], dst.at[block], sems.at[sem + zero])

        def chunk_of(step, outer, inner):
            return 2 * (step + _WIDTH * outer) + inner

        def start_step(step):
            part = lax.rem(step, _WIDTH)

            @pl.loop(0, CHUNKS // (2 * _WIDTH))
            def _(outer):
                for j in _WINDOW_ORDER:
                    pair = step + lax.rem(j - step + _WIDTH * PAIRS, _WIDTH)
                    for inner in range(2):
                        for which in range(2):
                            kv_copy(which, pair + which * _V_LEAD,
                                    chunk_of(part, outer, inner)).start(priority=which)

        def kv_list(which, steps):
            lead = which * _V_LEAD
            return [(kv_copy, which, pair, chunk_of(step % _WIDTH, outer, inner))
                    for step in steps
                    for outer in range(CHUNKS // (2 * _WIDTH))
                    for pair in [step + lead + (j - step) % _WIDTH for j in _WINDOW_ORDER]
                    if 0 <= pair < PAIRS
                    for inner in range(2)]

        def weight_list(src, dst, row, rows, col, cols, sem):
            n_cols = min(cols, E // 2)
            n_rows = _ROWS * _DH // n_cols
            return [(weight_copy, src, dst, r, n_rows, c, n_cols, sem)
                    for r in range(row, row + rows, n_rows)
                    for c in range(col, col + cols, n_cols)]

        def start_zipped(queues, begin, end, zero=0):
            for n in range(begin, end):
                for q in range(2):
                    copy, *args = queues[q][n]
                    copy(*args, zero=zero).start(priority=q)

        wq_all = weight_list(wq_hbm, wq_ref, 0, D, 0, E, WQ_SEM)

        def wq_list(bands):
            return [wq_all[16 * band + chunk_of(part, outer, inner)]
                    for part in range(4) for outer in range(2) for band in bands for inner in range(2)]

        head = (wq_list((3, 4, 5)) + wq_list((6, 7, 8)) + kv_list(0, range(1 - _WIDTH, 0)),
                wq_list((0, 1, 2)) + kv_list(1, range(1 - _WIDTH - _V_LEAD, 0)))
        assert len(head[0]) == len(head[1])

        last_step = PAIRS - _WIDTH - _V_LEAD
        tail = tuple(kv_list(which, range(last_step + 1, PAIRS)) for which in range(2))
        k_complete = {pair: n + 1 for n, (_, _, pair, _) in enumerate(tail[0])}
        wo_lists = [weight_list(wot_hbm, wot_ref, *piece, WO_SEM + u) for u, piece in enumerate(wo_pieces)]
        tail_len = sum(len(copies) for copies in (*tail, *wo_lists)) // 2
        free = sorted((n + q * _QUEUE1_LAG, q) for q in range(2) for n in range(len(tail[q]), tail_len))
        piece_end = []
        for copies in wo_lists:
            halves = [copies[:len(copies) // 2], copies[len(copies) // 2:]]
            end = 0
            for _ in copies:
                q = free.pop(0)[1]
                tail[q].append((halves[q] or halves[1 - q]).pop(0))
                end = max(end, len(tail[q]))
            piece_end.append(end)
        assert len(tail[0]) == len(tail[1]) == tail_len

        tail_steps = []
        started = 0
        for i in range(last_step + 1 - _LOOKAHEAD, PAIRS):
            end = k_complete.get(i + _LOOKAHEAD, started + CHUNKS // 2)
            tail_steps.append((i, started, end))
            started = end

        def project_queries(g):
            col = pl.multiple_of(g * (REP * _DH), REP * _DH)
            q = jnp.dot(x_ref[...], wq_ref[:, pl.ds(col, REP * _DH)], preferred_element_type=jnp.float32)
            q = q.astype(q_ref.dtype)
            for r in range(REP):
                for b in range(B):
                    q_ref[b, g, r * SQ:(r + 1) * SQ, :] = q[b * SQ:(b + 1) * SQ, r * _DH:(r + 1) * _DH]

        def attend(slot, b, g):
            s = lax.dot_general(q_ref[b, g], kv_ref[slot, 0], _NT, preferred_element_type=jnp.float32)
            m = jnp.max(s, axis=-1, keepdims=True)
            p = jnp.exp2((s - m) * exp2_scale)
            denom = jnp.sum(p, axis=-1, keepdims=True)
            o = jnp.dot(p.astype(kv_ref.dtype), kv_ref[slot, 1], preferred_element_type=jnp.float32)
            o = (o / denom).astype(att_ref.dtype)
            row = pl.multiple_of(b * SQ, SQ)
            for r in range(REP):
                att_ref[g * REP + r, pl.ds(row, SQ), :] = o[r * SQ:(r + 1) * SQ, :]

        def out_copy(n, col, cols):
            return pltpu.make_async_copy(out_ref.at[:, pl.ds(col, cols)], out_hbm.at[:, pl.ds(col, cols)],
                                         out_sems.at[n])

        x_copy = pltpu.make_async_copy(x_hbm, x_ref, x_sem)
        x_copy.start()

        @pl.loop(0, pl.cdiv(len(head[0]), CHUNKS))
        def _(i):
            for n, begin in enumerate(range(0, len(head[0]), CHUNKS)):
                @pl.when(i == n)
                def _():
                    start_zipped(head, begin, min(begin + CHUNKS, len(head[0])), zero=i - n)

        @pl.loop(0, _LOOKAHEAD)
        def _(step):
            start_step(step)

        x_copy.wait()
        pltpu.make_async_copy(wq_ref, wq_ref, sems.at[WQ_SEM]).wait()

        @pl.loop(0, PAIRS)
        def _(i):
            @pl.when(i + _LOOKAHEAD <= last_step)
            def _():
                start_step(i + _LOOKAHEAD)

            for n, begin, end in tail_steps:
                @pl.when(i == n)
                def _():
                    start_zipped(tail, begin, end, zero=i - n)

            @pl.when(i < HKV)
            def _():
                project_queries(i)

            slot = lax.rem(i, _SLOTS)
            pltpu.make_async_copy(kv_ref.at[slot], kv_ref.at[slot], sems.at[slot]).wait()
            attend(slot, lax.div(i, HKV), lax.rem(i, HKV))

        last_row, last_rows = wo_pieces[-1][:2]
        out_copies = [out_copy(0, 0, last_row), out_copy(1, last_row + last_rows, D - last_row - last_rows),
                      out_copy(2, last_row, last_rows)]
        acc = None
        for u, (row, rows, col, cols) in enumerate(wo_pieces):
            end = min(tail_len, max(started + 12, piece_end[u]))
            start_zipped(tail, started, end)
            started = end
            piece = wot_ref.at[pl.ds(row, rows), pl.ds(col, cols)]
            pltpu.make_async_copy(piece, piece, sems.at[WO_SEM + u]).wait()
            if u == len(wo_pieces) - 1:
                out_copies[0].start(priority=0)
                out_copies[1].start(priority=1)
            for h in range(col // _DH, (col + cols) // _DH):
                part = lax.dot_general(att_ref[h], wot_ref[row:row + rows, h * _DH:(h + 1) * _DH], _NT,
                                       preferred_element_type=jnp.float32)
                acc = part if acc is None else acc + part
            if col + cols == E:
                out_ref[:, row:row + rows] = acc.astype(out_ref.dtype)
                acc = None
        assert started == tail_len
        out_copies[2].start()
        for copy in out_copies:
            copy.wait()

    hbm = pl.BlockSpec(memory_space=pltpu.HBM)
    out = pl.pallas_call(
        kernel,
        out_shape=jax.ShapeDtypeStruct((M, D), x.dtype),
        in_specs=[hbm] * 5,
        out_specs=hbm,
        scratch_shapes=[
            pltpu.VMEM((M, D), x.dtype),
            pltpu.VMEM((D, E), wq.dtype),
            pltpu.VMEM((D, E), wo.dtype),
            pltpu.VMEM((_SLOTS, 2, W, _DH), k_cache.dtype),
            pltpu.VMEM((B, HKV, REP * SQ, _DH), k_cache.dtype),
            pltpu.VMEM((_HQ, M, _DH), wo.dtype),
            pltpu.VMEM((M, D), x.dtype),
            pltpu.SemaphoreType.DMA(()),
            pltpu.SemaphoreType.DMA((_SLOTS + 1 + len(wo_pieces),)),
            pltpu.SemaphoreType.DMA((3,)),
        ],
        compiler_params=pltpu.CompilerParams(
            vmem_limit_bytes=64 * 1024 * 1024,
            disable_bounds_checks=True,
            disable_semaphore_checks=True,
        ),
        name="sliding_block_cached_sampling",
    )(x.reshape(M, D), k_cache.reshape(PAIRS, SK, _DH), v_cache.reshape(PAIRS, SK, _DH), wq, wo.T)
    return out.reshape(B, SQ, D)
```

```python
import math

import jax
import jax.numpy as jnp
from jax import lax
import jax.experimental.pallas as pl
import jax.experimental.pallas.tpu as pltpu

_HQ, _DH = 32, 128
_NT = (((1,), (1,)), ((), ()))

_ROWS = 128
_WIDTH = 4
_WINDOW_ORDER = (0, 2, 1, 3)
_V_LEAD = 3
_LOOKAHEAD = 2
_SLOTS = 16
_QUEUE1_LAG = 30


@jax.jit
def pallas_standalone__sliding_block_cached__sampling_kernel(
    x: jax.Array,
    k_cache: jax.Array,
    v_cache: jax.Array,
    wq: jax.Array,
    wo: jax.Array,
):
    B, SQ, D = x.shape
    _, HKV, SK, _ = k_cache.shape
    W = min(4096, max(256, SK // 4))
    REP = _HQ // HKV
    M = B * SQ
    E = _HQ * _DH
    PAIRS = B * HKV
    CHUNKS = W // _ROWS
    assert CHUNKS == 16 and D == 576 and PAIRS >= _SLOTS
    assert _SLOTS > _LOOKAHEAD + _V_LEAD + _WIDTH
    exp2_scale = (_DH ** -0.5) * math.log2(math.e)

    wo_pieces = [
        (row, rows, E * a // 4, E * (b - a) // 4)
        for row, rows, cuts in ((512, 64, (0, 4)), (0, 128, (0, 4)), (128, 128, (0, 4)),
                                (256, 128, (0, 2, 4)), (384, 128, (0, 2, 3, 4)))
        for a, b in zip(cuts, cuts[1:])
    ]

    def kernel(x_hbm, k_hbm, v_hbm, wq_hbm, wot_hbm, out_hbm,
               x_ref, wq_ref, wot_ref, kv_ref, q_ref, att_ref, out_ref, x_sem, sems, out_sems):
        WQ_SEM, WO_SEM = _SLOTS, _SLOTS + 1

        def kv_copy(which, pair, chunk, zero=0):
            static = isinstance(pair, int)
            slot = pair % _SLOTS if static else lax.rem(pair, _SLOTS)
            row = chunk * _ROWS if static else pl.multiple_of(chunk * _ROWS, _ROWS)
            return pltpu.make_async_copy(
                (k_hbm, v_hbm)[which].at[pair, pl.ds(SK - W + row, _ROWS), :],
                kv_ref.at[slot, which, pl.ds(row, _ROWS), :],
                sems.at[slot + zero])

        def weight_copy(src, dst, row, rows, col, cols, sem, zero=0):
            block = (pl.ds(row, rows), pl.ds(col, cols))
            return pltpu.make_async_copy(src.at[block], dst.at[block], sems.at[sem + zero])

        def chunk_of(step, outer, inner):
            return 2 * (step + _WIDTH * outer) + inner

        def start_step(step):
            part = lax.rem(step, _WIDTH)

            @pl.loop(0, CHUNKS // (2 * _WIDTH))
            def _(outer):
                for j in _WINDOW_ORDER:
                    pair = step + lax.rem(j - step + _WIDTH * PAIRS, _WIDTH)
                    for inner in range(2):
                        for which in range(2):
                            kv_copy(which, pair + which * _V_LEAD,
                                    chunk_of(part, outer, inner)).start(priority=which)

        def kv_list(which, steps):
            lead = which * _V_LEAD
            return [(kv_copy, which, pair, chunk_of(step % _WIDTH, outer, inner))
                    for step in steps
                    for outer in range(CHUNKS // (2 * _WIDTH))
                    for pair in [step + lead + (j - step) % _WIDTH for j in _WINDOW_ORDER]
                    if 0 <= pair < PAIRS
                    for inner in range(2)]

        def weight_list(src, dst, row, rows, col, cols, sem, stride=64):
            n_cols = min(cols, E // 2)
            n_rows = _ROWS * _DH // n_cols
            return [(weight_copy, src, dst, r, n_rows, c, n_cols, sem)
                    for r in sorted(range(row, row + rows, n_rows), key=lambda r: (r // 64, r % stride))
                    for c in range(col, col + cols, n_cols)]

        def start_zipped(queues, begin, end, zero=0):
            for n in range(begin, end):
                for q in range(2):
                    copy, *args = queues[q][n]
                    copy(*args, zero=zero).start(priority=q)

        wq_all = weight_list(wq_hbm, wq_ref, 0, D, 0, E, WQ_SEM)

        def wq_list(bands):
            return [wq_all[16 * band + chunk_of(part, outer, inner)]
                    for part in range(4) for outer in range(2) for band in bands for inner in range(2)]

        head = (wq_list((3, 4, 5)) + wq_list((6, 7, 8)) + kv_list(0, range(1 - _WIDTH, 0)),
                wq_list((0, 1, 2)) + kv_list(1, range(1 - _WIDTH - _V_LEAD, 0)))
        assert len(head[0]) == len(head[1])

        last_step = PAIRS - _WIDTH - _V_LEAD
        tail = tuple(kv_list(which, range(last_step + 1, PAIRS)) for which in range(2))
        k_complete = {pair: n + 1 for n, (_, _, pair, _) in enumerate(tail[0])}
        wo_lists = [weight_list(wot_hbm, wot_ref, *piece, WO_SEM + u, stride=32 if piece[3] == E else 16)
                    for u, piece in enumerate(wo_pieces)]
        tail_len = sum(len(copies) for copies in (*tail, *wo_lists)) // 2
        free = sorted((n + q * _QUEUE1_LAG, q) for q in range(2) for n in range(len(tail[q]), tail_len))
        piece_end = []
        for copies in wo_lists:
            halves = [copies[:len(copies) // 2], copies[len(copies) // 2:]]
            end = 0
            for _ in copies:
                q = free.pop(0)[1]
                tail[q].append((halves[q] or halves[1 - q]).pop(0))
                end = max(end, len(tail[q]))
            piece_end.append(end)
        assert len(tail[0]) == len(tail[1]) == tail_len

        tail_steps = []
        started = 0
        for i in range(last_step + 1 - _LOOKAHEAD, PAIRS):
            end = k_complete.get(i + _LOOKAHEAD, started + CHUNKS // 2)
            tail_steps.append((i, started, end))
            started = end

        def project_queries(g):
            col = pl.multiple_of(g * (REP * _DH), REP * _DH)
            q = jnp.dot(x_ref[...], wq_ref[:, pl.ds(col, REP * _DH)], preferred_element_type=jnp.float32)
            q = q.astype(q_ref.dtype)
            for r in range(REP):
                for b in range(B):
                    q_ref[b, g, r * SQ:(r + 1) * SQ, :] = q[b * SQ:(b + 1) * SQ, r * _DH:(r + 1) * _DH]

        def attend(slot, b, g):
            s = lax.dot_general(q_ref[b, g], kv_ref[slot, 0], _NT, preferred_element_type=jnp.float32)
            m = jnp.max(s, axis=-1, keepdims=True)
            p = jnp.exp2((s - m) * exp2_scale)
            denom = jnp.sum(p, axis=-1, keepdims=True)
            o = jnp.dot(p.astype(kv_ref.dtype), kv_ref[slot, 1], preferred_element_type=jnp.float32)
            o = (o / denom).astype(att_ref.dtype)
            row = pl.multiple_of(b * SQ, SQ)
            for r in range(REP):
                att_ref[g * REP + r, pl.ds(row, SQ), :] = o[r * SQ:(r + 1) * SQ, :]

        def out_copy(n, col, cols):
            return pltpu.make_async_copy(out_ref.at[:, pl.ds(col, cols)], out_hbm.at[:, pl.ds(col, cols)],
                                         out_sems.at[n])

        x_copy = pltpu.make_async_copy(x_hbm, x_ref, x_sem)
        x_copy.start()

        @pl.loop(0, pl.cdiv(len(head[0]), CHUNKS))
        def _(i):
            for n, begin in enumerate(range(0, len(head[0]), CHUNKS)):
                @pl.when(i == n)
                def _():
                    start_zipped(head, begin, min(begin + CHUNKS, len(head[0])), zero=i - n)

        @pl.loop(0, _LOOKAHEAD)
        def _(step):
            start_step(step)

        x_copy.wait()
        pltpu.make_async_copy(wq_ref, wq_ref, sems.at[WQ_SEM]).wait()

        @pl.loop(0, PAIRS)
        def _(i):
            @pl.when(i + _LOOKAHEAD <= last_step)
            def _():
                start_step(i + _LOOKAHEAD)

            for n, begin, end in tail_steps:
                @pl.when(i == n)
                def _():
                    start_zipped(tail, begin, end, zero=i - n)

            @pl.when(i < HKV)
            def _():
                project_queries(i)

            slot = lax.rem(i, _SLOTS)
            pltpu.make_async_copy(kv_ref.at[slot], kv_ref.at[slot], sems.at[slot]).wait()
            attend(slot, lax.div(i, HKV), lax.rem(i, HKV))

        last_row, last_rows = wo_pieces[-1][:2]
        out_copies = [out_copy(0, 0, last_row), out_copy(1, last_row + last_rows, D - last_row - last_rows),
                      out_copy(2, last_row, last_rows)]
        acc = None
        for u, (row, rows, col, cols) in enumerate(wo_pieces):
            end = min(tail_len, max(started + 12, piece_end[u]))
            start_zipped(tail, started, end)
            started = end
            piece = wot_ref.at[pl.ds(row, rows), pl.ds(col, cols)]
            pltpu.make_async_copy(piece, piece, sems.at[WO_SEM + u]).wait()
            if u == len(wo_pieces) - 1:
                out_copies[0].start(priority=0)
                out_copies[1].start(priority=1)
            for h in range(col // _DH, (col + cols) // _DH):
                part = lax.dot_general(att_ref[h], wot_ref[row:row + rows, h * _DH:(h + 1) * _DH], _NT,
                                       preferred_element_type=jnp.float32)
                acc = part if acc is None else acc + part
            if col + cols == E:
                out_ref[:, row:row + rows] = acc.astype(out_ref.dtype)
                acc = None
        assert started == tail_len
        out_copies[2].start()
        for copy in out_copies:
            copy.wait()

    hbm = pl.BlockSpec(memory_space=pltpu.HBM)
    out = pl.pallas_call(
        kernel,
        out_shape=jax.ShapeDtypeStruct((M, D), x.dtype),
        in_specs=[hbm] * 5,
        out_specs=hbm,
        scratch_shapes=[
            pltpu.VMEM((M, D), x.dtype),
            pltpu.VMEM((D, E), wq.dtype),
            pltpu.VMEM((D, E), wo.dtype),
            pltpu.VMEM((_SLOTS, 2, W, _DH), k_cache.dtype),
            pltpu.VMEM((B, HKV, REP * SQ, _DH), k_cache.dtype),
            pltpu.VMEM((_HQ, M, _DH), wo.dtype),
            pltpu.VMEM((M, D), x.dtype),
            pltpu.SemaphoreType.DMA(()),
            pltpu.SemaphoreType.DMA((_SLOTS + 1 + len(wo_pieces),)),
            pltpu.SemaphoreType.DMA((3,)),
        ],
        compiler_params=pltpu.CompilerParams(
            vmem_limit_bytes=64 * 1024 * 1024,
            disable_bounds_checks=True,
            disable_semaphore_checks=True,
        ),
        name="sliding_block_cached_sampling",
    )(x.reshape(M, D), k_cache.reshape(PAIRS, SK, _DH), v_cache.reshape(PAIRS, SK, _DH), wq, wo.T)
    return out.reshape(B, SQ, D)
```

```python
import math

import jax
import jax.numpy as jnp
from jax import lax
import jax.experimental.pallas as pl
import jax.experimental.pallas.tpu as pltpu

_HQ, _DH = 32, 128
_NT = (((1,), (1,)), ((), ()))

_ROWS = 128
_WIDTH = 4
_WINDOW_ORDER = (0, 2, 1, 3)
_V_LEAD = 3
_LOOKAHEAD = 2
_SLOTS = 16
_QUEUE1_LAG = 34


@jax.jit
def pallas_standalone__sliding_block_cached__sampling_kernel(
    x: jax.Array,
    k_cache: jax.Array,
    v_cache: jax.Array,
    wq: jax.Array,
    wo: jax.Array,
):
    B, SQ, D = x.shape
    _, HKV, SK, _ = k_cache.shape
    W = min(4096, max(256, SK // 4))
    REP = _HQ // HKV
    M = B * SQ
    E = _HQ * _DH
    PAIRS = B * HKV
    CHUNKS = W // _ROWS
    assert CHUNKS == 16 and D == 576 and PAIRS >= _SLOTS
    assert _SLOTS > _LOOKAHEAD + _V_LEAD + _WIDTH
    exp2_scale = (_DH ** -0.5) * math.log2(math.e)

    wo_pieces = [
        (row, rows, E * a // 8, E * (b - a) // 8)
        for row, rows, cuts in ((512, 64, (0, 8)), (0, 128, (0, 8)), (128, 128, (0, 8)),
                                (256, 128, (0, 4, 8)), (384, 128, (0, 4, 6, 7, 8)))
        for a, b in zip(cuts, cuts[1:])
    ]

    def kernel(x_hbm, k_hbm, v_hbm, wq_hbm, wot_hbm, out_hbm,
               x_ref, wq_ref, wot_ref, kv_ref, q_ref, att_ref, out_ref, x_sem, sems, out_sems):
        WQ_SEM, WO_SEM = _SLOTS, _SLOTS + 1

        def kv_copy(which, pair, chunk, zero=0):
            static = isinstance(pair, int)
            slot = pair % _SLOTS if static else lax.rem(pair, _SLOTS)
            row = chunk * _ROWS if static else pl.multiple_of(chunk * _ROWS, _ROWS)
            return pltpu.make_async_copy(
                (k_hbm, v_hbm)[which].at[pair, pl.ds(SK - W + row, _ROWS), :],
                kv_ref.at[slot, which, pl.ds(row, _ROWS), :],
                sems.at[slot + zero])

        def weight_copy(src, dst, row, rows, col, cols, sem, zero=0):
            block = (pl.ds(row, rows), pl.ds(col, cols))
            return pltpu.make_async_copy(src.at[block], dst.at[block], sems.at[sem + zero])

        def chunk_of(step, outer, inner):
            return 2 * (step + _WIDTH * outer) + inner

        def start_step(step):
            part = lax.rem(step, _WIDTH)

            @pl.loop(0, CHUNKS // (2 * _WIDTH))
            def _(outer):
                for j in _WINDOW_ORDER:
                    pair = step + lax.rem(j - step + _WIDTH * PAIRS, _WIDTH)
                    for inner in range(2):
                        for which in range(2):
                            kv_copy(which, pair + which * _V_LEAD,
                                    chunk_of(part, outer, inner)).start(priority=which)

        def kv_list(which, steps):
            lead = which * _V_LEAD
            return [(kv_copy, which, pair, chunk_of(step % _WIDTH, outer, inner))
                    for step in steps
                    for outer in range(CHUNKS // (2 * _WIDTH))
                    for pair in [step + lead + (j - step) % _WIDTH for j in _WINDOW_ORDER]
                    if 0 <= pair < PAIRS
                    for inner in range(2)]

        def weight_list(src, dst, row, rows, col, cols, sem, stride=64):
            n_cols = min(cols, E // 2)
            n_rows = _ROWS * _DH // n_cols
            return [(weight_copy, src, dst, r, n_rows, c, n_cols, sem)
                    for r in sorted(range(row, row + rows, n_rows), key=lambda r: (r // 64, r % stride))
                    for c in range(col, col + cols, n_cols)]

        def start_zipped(queues, begin, end, zero=0):
            for n in range(begin, end):
                for q in range(2):
                    copy, *args = queues[q][n]
                    copy(*args, zero=zero).start(priority=q)

        wq_all = weight_list(wq_hbm, wq_ref, 0, D, 0, E, WQ_SEM)

        def wq_list(bands):
            return [wq_all[16 * band + chunk_of(part, outer, inner)]
                    for part in range(4) for outer in range(2) for band in bands for inner in range(2)]

        head = (wq_list((3, 4, 5)) + wq_list((6, 7, 8)) + kv_list(0, range(1 - _WIDTH, 0)),
                wq_list((0, 1, 2)) + kv_list(1, range(1 - _WIDTH - _V_LEAD, 0)))
        assert len(head[0]) == len(head[1])

        last_step = PAIRS - _WIDTH - _V_LEAD
        tail = tuple(kv_list(which, range(last_step + 1, PAIRS)) for which in range(2))
        k_complete = {pair: n + 1 for n, (_, _, pair, _) in enumerate(tail[0])}
        wo_lists = [weight_list(wot_hbm, wot_ref, *piece, WO_SEM + u, stride=32 if piece[3] == E else 16)
                    for u, piece in enumerate(wo_pieces)]
        tail_len = sum(len(copies) for copies in (*tail, *wo_lists)) // 2
        free = sorted((n + q * _QUEUE1_LAG, q) for q in range(2) for n in range(len(tail[q]), tail_len))
        piece_end = []
        for copies in wo_lists:
            halves = [copies[:len(copies) // 2], copies[len(copies) // 2:]]
            end = 0
            for _ in copies:
                q = free.pop(0)[1]
                tail[q].append((halves[q] or halves[1 - q]).pop(0))
                end = max(end, len(tail[q]))
            piece_end.append(end)
        assert len(tail[0]) == len(tail[1]) == tail_len

        tail_steps = []
        started = 0
        for i in range(last_step + 1 - _LOOKAHEAD, PAIRS):
            end = k_complete.get(i + _LOOKAHEAD, started + CHUNKS // 2)
            tail_steps.append((i, started, end))
            started = end

        def project_queries(g):
            col = pl.multiple_of(g * (REP * _DH), REP * _DH)
            q = jnp.dot(x_ref[...], wq_ref[:, pl.ds(col, REP * _DH)], preferred_element_type=jnp.float32)
            q = q.astype(q_ref.dtype)
            for r in range(REP):
                for b in range(B):
                    q_ref[b, g, r * SQ:(r + 1) * SQ, :] = q[b * SQ:(b + 1) * SQ, r * _DH:(r + 1) * _DH]

        def attend(slot, b, g):
            s = lax.dot_general(q_ref[b, g], kv_ref[slot, 0], _NT, preferred_element_type=jnp.float32)
            m = jnp.max(s, axis=-1, keepdims=True)
            p = jnp.exp2((s - m) * exp2_scale)
            denom = jnp.sum(p, axis=-1, keepdims=True)
            o = jnp.dot(p.astype(kv_ref.dtype), kv_ref[slot, 1], preferred_element_type=jnp.float32)
            o = (o / denom).astype(att_ref.dtype)
            row = pl.multiple_of(b * SQ, SQ)
            for r in range(REP):
                att_ref[g * REP + r, pl.ds(row, SQ), :] = o[r * SQ:(r + 1) * SQ, :]

        def out_copy(n, col, cols):
            return pltpu.make_async_copy(out_ref.at[:, pl.ds(col, cols)], out_hbm.at[:, pl.ds(col, cols)],
                                         out_sems.at[n])

        x_copy = pltpu.make_async_copy(x_hbm, x_ref, x_sem)
        x_copy.start()

        @pl.loop(0, pl.cdiv(len(head[0]), CHUNKS))
        def _(i):
            for n, begin in enumerate(range(0, len(head[0]), CHUNKS)):
                @pl.when(i == n)
                def _():
                    start_zipped(head, begin, min(begin + CHUNKS, len(head[0])), zero=i - n)

        @pl.loop(0, _LOOKAHEAD)
        def _(step):
            start_step(step)

        x_copy.wait()
        pltpu.make_async_copy(wq_ref, wq_ref, sems.at[WQ_SEM]).wait()

        @pl.loop(0, PAIRS)
        def _(i):
            @pl.when(i + _LOOKAHEAD <= last_step)
            def _():
                start_step(i + _LOOKAHEAD)

            for n, begin, end in tail_steps:
                @pl.when(i == n)
                def _():
                    start_zipped(tail, begin, end, zero=i - n)

            @pl.when(i < HKV)
            def _():
                project_queries(i)

            slot = lax.rem(i, _SLOTS)
            pltpu.make_async_copy(kv_ref.at[slot], kv_ref.at[slot], sems.at[slot]).wait()
            attend(slot, lax.div(i, HKV), lax.rem(i, HKV))

        last_row, last_rows = wo_pieces[-1][:2]
        out_copies = [out_copy(0, 0, last_row), out_copy(1, last_row + last_rows, D - last_row - last_rows),
                      out_copy(2, last_row, last_rows)]
        acc = [None, None]
        for u, (row, rows, col, cols) in enumerate(wo_pieces):
            end = min(tail_len, max(started + 12, piece_end[u]))
            start_zipped(tail, started, end)
            started = end
            piece = wot_ref.at[pl.ds(row, rows), pl.ds(col, cols)]
            pltpu.make_async_copy(piece, piece, sems.at[WO_SEM + u]).wait()
            if u == len(wo_pieces) - 1:
                out_copies[0].start(priority=0)
                out_copies[1].start(priority=1)
            for h in range(col // _DH, (col + cols) // _DH):
                w = wot_ref[row:row + rows, h * _DH:(h + 1) * _DH]
                for half in range(2):
                    part = lax.dot_general(att_ref[h, half * M // 2:(half + 1) * M // 2], w, _NT,
                                           preferred_element_type=jnp.float32)
                    acc[half] = part if acc[half] is None else acc[half] + part
            if col + cols == E:
                for half in range(2):
                    out_ref[half * M // 2:(half + 1) * M // 2, row:row + rows] = acc[half].astype(out_ref.dtype)
                acc = [None, None]
        assert started == tail_len
        out_copies[2].start()
        for copy in out_copies:
            copy.wait()

    hbm = pl.BlockSpec(memory_space=pltpu.HBM)
    out = pl.pallas_call(
        kernel,
        out_shape=jax.ShapeDtypeStruct((M, D), x.dtype),
        in_specs=[hbm] * 5,
        out_specs=hbm,
        scratch_shapes=[
            pltpu.VMEM((M, D), x.dtype),
            pltpu.VMEM((D, E), wq.dtype),
            pltpu.VMEM((D, E), wo.dtype),
            pltpu.VMEM((_SLOTS, 2, W, _DH), k_cache.dtype),
            pltpu.VMEM((B, HKV, REP * SQ, _DH), k_cache.dtype),
            pltpu.VMEM((_HQ, M, _DH), wo.dtype),
            pltpu.VMEM((M, D), x.dtype),
            pltpu.SemaphoreType.DMA(()),
            pltpu.SemaphoreType.DMA((_SLOTS + 1 + len(wo_pieces),)),
            pltpu.SemaphoreType.DMA((3,)),
        ],
        compiler_params=pltpu.CompilerParams(
            vmem_limit_bytes=64 * 1024 * 1024,
            disable_bounds_checks=True,
            disable_semaphore_checks=True,
            flags={"XLA_TPU_RESCHEDULE_DMA_DONES": True},
        ),
        name="sliding_block_cached_sampling",
    )(x.reshape(M, D), k_cache.reshape(PAIRS, SK, _DH), v_cache.reshape(PAIRS, SK, _DH), wq, wo.T)
    return out.reshape(B, SQ, D)
```

```python
import math

import jax
import jax.numpy as jnp
from jax import lax
import jax.experimental.pallas as pl
import jax.experimental.pallas.tpu as pltpu

_HQ, _DH = 32, 128
_NT = (((1,), (1,)), ((), ()))

_ROWS = 128
_WIDTH = 4
_WINDOW_ORDER = (0, 2, 1, 3)
_V_LEAD = 3
_LOOKAHEAD = 2
_SLOTS = 16
_QUEUE1_LAG = 34


@jax.jit
def pallas_standalone__sliding_block_cached__sampling_kernel(
    x: jax.Array,
    k_cache: jax.Array,
    v_cache: jax.Array,
    wq: jax.Array,
    wo: jax.Array,
):
    B, SQ, D = x.shape
    _, HKV, SK, _ = k_cache.shape
    W = min(4096, max(256, SK // 4))
    REP = _HQ // HKV
    M = B * SQ
    E = _HQ * _DH
    PAIRS = B * HKV
    CHUNKS = W // _ROWS
    assert CHUNKS == 16 and D == 576 and PAIRS >= _SLOTS
    assert _SLOTS > _LOOKAHEAD + _V_LEAD + _WIDTH
    exp2_scale = (_DH ** -0.5) * math.log2(math.e)

    wo_pieces = [
        (row, rows, E * a // 8, E * (b - a) // 8)
        for row, rows, cuts in ((512, 64, (0, 8)), (0, 128, (0, 8)), (128, 128, (0, 8)),
                                (256, 128, (0, 4, 8)), (384, 128, (0, 4, 6, 7, 8)))
        for a, b in zip(cuts, cuts[1:])
    ]

    def kernel(x_hbm, k_hbm, v_hbm, wq_hbm, wot_hbm, out_hbm,
               x_ref, wq_ref, wot_ref, kv_ref, q_ref, att_ref, out_ref, x_sem, sems, out_sems):
        WQ_SEM, WO_SEM = _SLOTS, _SLOTS + 1

        def kv_copy(which, pair, chunk, zero=0):
            static = isinstance(pair, int)
            slot = pair % _SLOTS if static else lax.rem(pair, _SLOTS)
            row = chunk * _ROWS if static else pl.multiple_of(chunk * _ROWS, _ROWS)
            return pltpu.make_async_copy(
                (k_hbm, v_hbm)[which].at[pair, pl.ds(SK - W + row, _ROWS), :],
                kv_ref.at[slot, which, pl.ds(row, _ROWS), :],
                sems.at[slot + zero])

        def weight_copy(src, dst, row, rows, col, cols, sem, zero=0):
            block = (pl.ds(row, rows), pl.ds(col, cols))
            return pltpu.make_async_copy(src.at[block], dst.at[block], sems.at[sem + zero])

        def chunk_of(step, outer, inner):
            return 2 * (step + _WIDTH * outer) + inner

        def start_step(step):
            part = lax.rem(step, _WIDTH)

            @pl.loop(0, CHUNKS // (2 * _WIDTH))
            def _(outer):
                for j in _WINDOW_ORDER:
                    pair = step + lax.rem(j - step + _WIDTH * PAIRS, _WIDTH)
                    for inner in range(2):
                        for which in range(2):
                            kv_copy(which, pair + which * _V_LEAD,
                                    chunk_of(part, outer, inner)).start(priority=which)

        def kv_list(which, steps):
            lead = which * _V_LEAD
            return [(kv_copy, which, pair, chunk_of(step % _WIDTH, outer, inner))
                    for step in steps
                    for outer in range(CHUNKS // (2 * _WIDTH))
                    for pair in [step + lead + (j - step) % _WIDTH for j in _WINDOW_ORDER]
                    if 0 <= pair < PAIRS
                    for inner in range(2)]

        def weight_list(src, dst, row, rows, col, cols, sem, stride=64):
            n_cols = min(cols, E // 2)
            n_rows = _ROWS * _DH // n_cols
            return [(weight_copy, src, dst, r, n_rows, c, n_cols, sem)
                    for r in sorted(range(row, row + rows, n_rows), key=lambda r: (r // 64, r % stride))
                    for c in range(col, col + cols, n_cols)]

        def start_zipped(queues, begin, end, zero=0):
            for n in range(begin, end):
                for q in range(2):
                    copy, *args = queues[q][n]
                    copy(*args, zero=zero).start(priority=q)

        wq_all = weight_list(wq_hbm, wq_ref, 0, D, 0, E, WQ_SEM)

        def wq_list(bands):
            return [wq_all[16 * band + chunk_of(part, outer, inner)]
                    for part in range(4) for outer in range(2) for band in bands for inner in range(2)]

        head = (wq_list((3, 4, 5)) + wq_list((6, 7, 8)) + kv_list(0, range(1 - _WIDTH, 0)),
                wq_list((0, 1, 2)) + kv_list(1, range(1 - _WIDTH - _V_LEAD, 0)))
        assert len(head[0]) == len(head[1])

        last_step = PAIRS - _WIDTH - _V_LEAD
        tail = tuple(kv_list(which, range(last_step + 1, PAIRS)) for which in range(2))
        k_complete = {pair: n + 1 for n, (_, _, pair, _) in enumerate(tail[0])}
        wo_lists = [weight_list(wot_hbm, wot_ref, *piece, WO_SEM + u, stride=32 if piece[3] == E else 16)
                    for u, piece in enumerate(wo_pieces)]
        tail_len = sum(len(copies) for copies in (*tail, *wo_lists)) // 2
        free = sorted((n + q * _QUEUE1_LAG, q) for q in range(2) for n in range(len(tail[q]), tail_len))
        piece_end = []
        for copies in wo_lists:
            halves = [copies[:len(copies) // 2], copies[len(copies) // 2:]]
            end = 0
            for _ in copies:
                q = free.pop(0)[1]
                tail[q].append((halves[q] or halves[1 - q]).pop(0))
                end = max(end, len(tail[q]))
            piece_end.append(end)
        assert len(tail[0]) == len(tail[1]) == tail_len

        tail_steps = []
        started = 0
        for i in range(last_step + 1 - _LOOKAHEAD, PAIRS):
            end = k_complete.get(i + _LOOKAHEAD, started + 3 * CHUNKS // 4)
            tail_steps.append((i, started, end))
            started = end

        def project_queries(g):
            col = pl.multiple_of(g * (REP * _DH), REP * _DH)
            q = jnp.dot(x_ref[...], wq_ref[:, pl.ds(col, REP * _DH)], preferred_element_type=jnp.float32)
            q = q.astype(q_ref.dtype)
            for r in range(REP):
                for b in range(B):
                    q_ref[b, g, r * SQ:(r + 1) * SQ, :] = q[b * SQ:(b + 1) * SQ, r * _DH:(r + 1) * _DH]

        def attend(slot, b, g):
            s = lax.dot_general(q_ref[b, g], kv_ref[slot, 0], _NT, preferred_element_type=jnp.float32)
            m = jnp.max(s, axis=-1, keepdims=True)
            p = jnp.exp2((s - m) * exp2_scale)
            denom = jnp.sum(p, axis=-1, keepdims=True)
            o = jnp.dot(p.astype(kv_ref.dtype), kv_ref[slot, 1], preferred_element_type=jnp.float32)
            o = (o / denom).astype(att_ref.dtype)
            row = pl.multiple_of(b * SQ, SQ)
            for r in range(REP):
                att_ref[g * REP + r, pl.ds(row, SQ), :] = o[r * SQ:(r + 1) * SQ, :]

        def out_copy(n, col, cols):
            return pltpu.make_async_copy(out_ref.at[:, pl.ds(col, cols)], out_hbm.at[:, pl.ds(col, cols)],
                                         out_sems.at[n])

        x_copy = pltpu.make_async_copy(x_hbm, x_ref, x_sem)
        x_copy.start()

        @pl.loop(0, pl.cdiv(len(head[0]), CHUNKS))
        def _(i):
            for n, begin in enumerate(range(0, len(head[0]), CHUNKS)):
                @pl.when(i == n)
                def _():
                    start_zipped(head, begin, min(begin + CHUNKS, len(head[0])), zero=lax.div(i, PAIRS))

        @pl.loop(0, _LOOKAHEAD)
        def _(step):
            start_step(step)

        x_copy.wait()
        pltpu.make_async_copy(wq_ref, wq_ref, sems.at[WQ_SEM]).wait()

        @pl.loop(0, PAIRS)
        def _(i):
            @pl.when(i + _LOOKAHEAD <= last_step)
            def _():
                start_step(i + _LOOKAHEAD)

            for n, begin, end in tail_steps:
                @pl.when(i == n)
                def _():
                    start_zipped(tail, begin, end, zero=lax.div(i, PAIRS))

            @pl.when(i < HKV)
            def _():
                project_queries(i)

            slot = lax.rem(i, _SLOTS)
            pltpu.make_async_copy(kv_ref.at[slot], kv_ref.at[slot], sems.at[slot]).wait()
            attend(slot, lax.div(i, HKV), lax.rem(i, HKV))

        last_row, last_rows = wo_pieces[-1][:2]
        out_copies = [out_copy(0, 0, last_row), out_copy(1, last_row + last_rows, D - last_row - last_rows),
                      out_copy(2, last_row, last_rows)]
        acc = [None, None]
        for u, (row, rows, col, cols) in enumerate(wo_pieces):
            end = min(tail_len, max(started + CHUNKS, piece_end[u]))
            start_zipped(tail, started, end)
            started = end
            piece = wot_ref.at[pl.ds(row, rows), pl.ds(col, cols)]
            pltpu.make_async_copy(piece, piece, sems.at[WO_SEM + u]).wait()
            if u == len(wo_pieces) - 1:
                out_copies[0].start(priority=0)
                out_copies[1].start(priority=1)
            for h in range(col // _DH, (col + cols) // _DH):
                w = wot_ref[row:row + rows, h * _DH:(h + 1) * _DH]
                for half in range(2):
                    part = lax.dot_general(att_ref[h, half * M // 2:(half + 1) * M // 2], w, _NT,
                                           preferred_element_type=jnp.float32)
                    acc[half] = part if acc[half] is None else acc[half] + part
            if col + cols == E:
                for half in range(2):
                    out_ref[half * M // 2:(half + 1) * M // 2, row:row + rows] = acc[half].astype(out_ref.dtype)
                acc = [None, None]
        assert started == tail_len
        out_copies[2].start()
        for copy in out_copies:
            copy.wait()

    hbm = pl.BlockSpec(memory_space=pltpu.HBM)
    out = pl.pallas_call(
        kernel,
        out_shape=jax.ShapeDtypeStruct((M, D), x.dtype),
        in_specs=[hbm] * 5,
        out_specs=hbm,
        scratch_shapes=[
            pltpu.VMEM((M, D), x.dtype),
            pltpu.VMEM((D, E), wq.dtype),
            pltpu.VMEM((D, E), wo.dtype),
            pltpu.VMEM((_SLOTS, 2, W, _DH), k_cache.dtype),
            pltpu.VMEM((B, HKV, REP * SQ, _DH), k_cache.dtype),
            pltpu.VMEM((_HQ, M, _DH), wo.dtype),
            pltpu.VMEM((M, D), x.dtype),
            pltpu.SemaphoreType.DMA(()),
            pltpu.SemaphoreType.DMA((_SLOTS + 1 + len(wo_pieces),)),
            pltpu.SemaphoreType.DMA((3,)),
        ],
        compiler_params=pltpu.CompilerParams(
            vmem_limit_bytes=64 * 1024 * 1024,
            disable_bounds_checks=True,
            disable_semaphore_checks=True,
            flags={"XLA_TPU_RESCHEDULE_DMA_DONES": True},
        ),
        name="sliding_block_cached_sampling",
    )(x.reshape(M, D), k_cache.reshape(PAIRS, SK, _DH), v_cache.reshape(PAIRS, SK, _DH), wq, wo.T)
    return out.reshape(B, SQ, D)
```
